```python
import os as _os
_os.environ.setdefault("JAX_PLATFORMS", "cpu")
import jax
import jax.numpy as jnp

def _softmax(x, axis=-1):
    return jax.nn.softmax(x, axis=axis)
def _gelu(x):
    return jax.nn.gelu(x, approximate=True)
def _silu(x):
    return jax.nn.silu(x)
def _sigmoid(x):
    return jax.nn.sigmoid(x)
def _layernorm(x, axis=-1, eps=1e-5):
    m = jnp.mean(x, axis=axis, keepdims=True)
    v = jnp.var(x, axis=axis, keepdims=True)
    return (x - m) / jnp.sqrt(v + eps)
def _scatter_add(tgt, idx, src, axis=0):
    return tgt.at[idx].add(src)
def _segment_sum(src, seg, n):
    return jax.ops.segment_sum(src, seg, n)
class _Rng:
    def __init__(self, key):
        self._k = key
    def _next(self):
        self._k, sub = jax.random.split(self._k)
        return sub
    def normal(self, shape):
        return jax.random.normal(self._next(), shape, dtype=jnp.bfloat16)
    def randint(self, lo, hi, shape):
        return jax.random.randint(self._next(), shape, lo, hi, dtype=jnp.int32)
    def uniform(self, shape, lo=0.0, hi=1.0):
        return jax.random.uniform(self._next(), shape, jnp.bfloat16, lo, hi)
    def permutation(self, n):
        return jax.random.permutation(self._next(), n)


kernel_name = 'gated_mix__mha_block__mha_block__prompt'

def setup_inputs():
    _rng = _Rng(jax.random.key(int.from_bytes(__import__("os").urandom(4), "little")))
    _w = (lambda a: (lambda t: t.astype(jnp.bfloat16) if jnp.issubdtype(t.dtype, jnp.floating) else t)(jnp.asarray(a)))
    def _A_setup():
        B, S, D, H = 1, 2048, 448, 16
        return {
            "x": _w((lambda *s: _rng.normal(s) * 0.05)(B, S, D)),
            "wqkv": _w((lambda *s: _rng.normal(s) * 0.4)(D, 3 * D)),
            "wo": _w((lambda *s: _rng.normal(s) * 0.05)(D, D)),
        }
    _A_in = _A_setup()

    def _B_setup():
        B, S, D, H = 1, 2048, 448, 16
        return {
            "x": _w((lambda *s: _rng.normal(s) * 0.05)(B, S, D)),
            "wqkv": _w((lambda *s: _rng.normal(s) * 0.4)(D, 3 * D)),
            "wo": _w((lambda *s: _rng.normal(s) * 0.05)(D, D)),
        }
    _B_in = _B_setup()

    return {
        "A_x": _A_in["x"],
        "A_wqkv": _A_in["wqkv"],
        "A_wo": _A_in["wo"],
        "B_x": _B_in["x"],
        "B_wqkv": _B_in["wqkv"],
        "B_wo": _B_in["wo"],
        "gate_w": _w((lambda *s: _rng.normal(s) * 0.05)(448) * 16.0),
    }

def reference(A_x, A_wqkv, A_wo, B_x, B_wqkv, B_wo, gate_w):
    def _A_ref(x, wqkv, wo):
        B, S, D = x.shape
        H = 16
        Dh = D // H
        qkv = (lambda x, *d: x.transpose(*d))((x @ wqkv).reshape(B, S, 3, H, Dh), 2, 0, 3, 1, 4)
        q, k, v = qkv[0], qkv[1], qkv[2]
        scores = jnp.einsum("bhqd,bhkd->bhqk", q, k) * (Dh ** -0.5)
        p = _softmax(scores, axis=-1)
        o = jnp.einsum("bhqk,bhkd->bhqd", p, v)
        return (lambda x, *d: x.transpose(*d))(o, 0, 2, 1, 3).reshape(B, S, D) @ wo

    def _B_ref(x, wqkv, wo):
        B, S, D = x.shape
        H = 16
        Dh = D // H
        qkv = (lambda x, *d: x.transpose(*d))((x @ wqkv).reshape(B, S, 3, H, Dh), 2, 0, 3, 1, 4)
        q, k, v = qkv[0], qkv[1], qkv[2]
        scores = jnp.einsum("bhqd,bhkd->bhqk", q, k) * (Dh ** -0.5)
        p = _softmax(scores, axis=-1)
        o = jnp.einsum("bhqk,bhkd->bhqd", p, v)
        return (lambda x, *d: x.transpose(*d))(o, 0, 2, 1, 3).reshape(B, S, D) @ wo

    x = A_x
    g = _sigmoid((x * gate_w).sum(-1, keepdims=True))
    a = _A_ref(x, A_wqkv, A_wo)
    b = _B_ref(x, B_wqkv, B_wo)
    return g * a + (1 - g) * b
```

```python
import functools
import numpy as np
import jax
import jax.numpy as jnp
import jax.experimental.pallas as pl
import jax.experimental.pallas.tpu as pltpu

S, D, H, DH = 2048, 448, 16, 28
HP = 32
TQ = 512
KC = 128
G = 4
LASTSWAP = 1
PW = 512
PRO_LOOP = False
NQ = S // TQ
NJ = S // KC
NI = 2 * H * NQ
NB = NI // G
QSCALE = float(DH ** -0.5 * np.log2(np.e))
NT = (((1,), (1,)), ((), ()))
F32 = jnp.float32
BF16 = jnp.bfloat16


def _kernel(x_hbm, wa_hbm, woa_hbm, wb_hbm, wob_hbm, gw_hbm, out_hbm,
            x_ref, w_ref, wo_ref, gw_ref, out_ref, sems, osems,
            wb16_ref, wot_ref, qt_ref, k_ref, vt_ref, at_ref, part_ref,
            g_ref, m_ref, *sbufs):
    cp_w = [pltpu.make_async_copy(w, w_ref.at[i], sems.at[i]) for i, w in enumerate((wa_hbm, wb_hbm))]
    cp_x = [pltpu.make_async_copy(x_hbm.at[0, :, pl.ds(c * TQ, TQ)], x_ref.at[:, pl.ds(c * TQ, TQ)],
                                  sems.at[2 + c]) for c in range(NQ)]
    cp_g = pltpu.make_async_copy(gw_hbm, gw_ref, sems.at[2 + NQ])
    cp_wo = [pltpu.make_async_copy(w, wo_ref.at[pl.ds(i * D, D), :], sems.at[3 + NQ + i])
             for i, w in enumerate((woa_hbm, wob_hbm))]
    cp_w[0].start()
    cp_g.start()
    cp_x[0].start()

    def prep_w(blk):
        for j in range(11):
            c0 = j * 128
            cw = min(128, 3 * D - c0)
            wb16_ref[blk, pl.ds(c0, cw), :] = w_ref[blk, :, pl.ds(c0, cw)].astype(F32).T.astype(BF16)

    zpad = jnp.zeros((HP - DH, PW), F32)
    opad = jnp.where(jax.lax.broadcasted_iota(jnp.int32, (HP - DH, PW), 0) == 0, 1.0, 0.0).astype(F32)

    def proj_unit(blk, c, gate=True):
        for n in range(TQ // PW):
            q0 = c * TQ + n * PW
            q0 = q0 if isinstance(c, int) else pl.multiple_of(q0, PW)
            xs = x_ref[:, pl.ds(q0, PW)]
            k = jnp.dot(wb16_ref[blk, pl.ds(D, D), :], xs, preferred_element_type=F32)
            for hg in range(H // 4):
                kg = jnp.concatenate(
                    [z for h in range(4 * hg, 4 * hg + 4) for z in (k[h * DH:(h + 1) * DH], zpad)], axis=0)
                kg = kg.T.astype(BF16)
                for hh in range(4):
                    k_ref[blk * H + 4 * hg + hh, pl.ds(q0, PW), :] = kg[:, hh * HP:(hh + 1) * HP]
            gw16 = jnp.broadcast_to(gw_ref[...].reshape(1, D), (16, D))
            gpre = jnp.dot(gw16, xs, preferred_element_type=F32)[0:8, :]
            gate = 1.0 / (1.0 + jnp.exp(-gpre))
            g_ref[0, :, pl.ds(q0, PW)] = gate
            g_ref[1, :, pl.ds(q0, PW)] = 1.0 - gate
            q = jnp.dot(wb16_ref[blk, pl.ds(0, D), :], xs, preferred_element_type=F32) * QSCALE
            v = jnp.dot(wb16_ref[blk, pl.ds(2 * D, D), :], xs, preferred_element_type=F32)
            for h in range(H):
                qh = jnp.concatenate([q[h * DH:(h + 1) * DH], zpad], axis=0)
                qt_ref[blk * H + h, :, pl.ds(q0, PW)] = qh.astype(BF16)
                vh = jnp.concatenate([v[h * DH:(h + 1) * DH], opad], axis=0)
                vt_ref[blk * H + h, :, pl.ds(q0, PW)] = vh.astype(BF16)

    cp_w[0].wait()
    cp_w[1].start()
    for c in cp_x[1:]:
        c.start()
    prep_w(0)
    cp_g.wait()
    cp_x[0].wait()
    proj_unit(0, 0)
    cp_w[1].wait()
    for c in cp_x[1:]:
        c.wait()
    for c in cp_wo:
        c.start()
    proj_unit(0, 1)
    prep_w(1)

    def pbody(t, carry):
        proj_unit(t // NQ, t % NQ)
        return carry
    jax.lax.fori_loop(2, 2 * NQ, pbody, 0)

    def idx(i):
        h = 2 * (i // (2 * NQ)) + i % 2
        return h, pl.multiple_of((i // 2) % NQ * TQ, TQ)

    def qk_chunk(h, qt, j, buf):
        s = jnp.dot(k_ref[h, pl.ds(j * KC, KC), :], qt, preferred_element_type=F32)
        buf[pl.ds(j * KC, KC), :] = s
        return s.reshape(KC // 8, 8, TQ).max(axis=0)

    def pv_chunk(h, m, j, buf):
        s = buf[pl.ds(j * KC, KC), :]
        p = jnp.exp2(s - m).astype(BF16)
        return jnp.dot(vt_ref[h, :, pl.ds(j * KC, KC)], p, preferred_element_type=F32)

    bufs = sbufs
    for c in cp_wo:
        c.wait()

    def prologue(g, carry):
        h0, q00 = idx(g)
        qt = qt_ref[h0, :, pl.ds(q00, TQ)]
        m = None
        for j in range(NJ):
            mm = qk_chunk(h0, qt, j, bufs[0].at[g])
            m = mm if m is None else jnp.maximum(m, mm)
        m_ref[0, g] = m
        return carry
    if PRO_LOOP:
        jax.lax.fori_loop(0, G - 1, prologue, 0)
        prologue(G - 1, 0)
    else:
        for g in range(G):
            prologue(g, 0)
    for j in range(2 * D // 128):
        wot_ref[:, pl.ds(j * 128, 128)] = wo_ref[pl.ds(j * 128, 128), :].astype(F32).T.astype(BF16)

    QF = NQ - G // 2
    KS = (2 * H - 2 * (-(-G // (2 * NQ)))) * DH // 128 * 128

    def at_flat(c0, w, r0, n):
        lo, hi = r0 // (2 * DH), -(-(r0 + n) // (2 * DH))
        a = at_ref[pl.ds(lo, hi - lo), :, pl.ds(c0, w)].reshape((hi - lo) * 2 * DH, w)
        return a[r0 - lo * 2 * DH:r0 - lo * 2 * DH + n].astype(BF16)

    def block(b, par, do_qk=True):
        for g in range(G):
            i = b * G + g
            h, q0 = idx(i)
            cur = bufs[par].at[g]
            nxt = bufs[1 - par].at[g]
            if do_qk:
                hn, qn = idx(i + G)
                qt = qt_ref[hn, :, pl.ds(qn, TQ)]
            m = jnp.max(m_ref[par, g], axis=0, keepdims=True)
            mn = None
            acc = None
            for j in range(NJ):
                qk_first = g < G - LASTSWAP
                if do_qk and qk_first:
                    mm = qk_chunk(hn, qt, j, nxt)
                    mn = mm if mn is None else jnp.maximum(mn, mm)
                pv = pv_chunk(h, m, j, cur)
                acc = pv if acc is None else acc + pv
                if do_qk and not qk_first:
                    mm = qk_chunk(hn, qt, j, nxt)
                    mn = mm if mn is None else jnp.maximum(mn, mm)
                npc = S // 128 // G
                if not do_qk and j % (NJ // npc) == 0:
                    c0 = (g * npc + j // (NJ // npc)) * 128
                    if c0 < QF * TQ:
                        a = at_flat(c0, 128, 0, 2 * D)
                        out_ref[:, pl.ds(c0, 128)] = jnp.dot(
                            wot_ref[...], a, preferred_element_type=F32).astype(out_ref.dtype)
                    else:
                        a = at_flat(c0, 128, 0, KS)
                        part_ref[:, pl.ds(c0 - QF * TQ, 128)] = jnp.dot(
                            wot_ref[:, pl.ds(0, KS)], a, preferred_element_type=F32)
            gt = g_ref[h // H, 0:1, pl.ds(q0, TQ)]
            o = acc[0:DH] * (gt / acc[DH:DH + 1, :])
            hpar = g % 2
            at_ref[h // 2, pl.ds(hpar * DH, DH), pl.ds(q0, TQ)] = o
            if do_qk:
                m_ref[1 - par, g] = mn

    def body(b, c):
        @pl.when(b % 2 == 0)
        def _():
            block(b, 0)

        @pl.when(b % 2 == 1)
        def _():
            block(b, 1)
        return c
    jax.lax.fori_loop(0, NB - 1, body, 0)
    block(NB - 1, (NB - 1) % 2, do_qk=False)

    cp_o = [pltpu.make_async_copy(out_ref.at[:, pl.ds(c * TQ, TQ)], out_hbm.at[0, :, pl.ds(c * TQ, TQ)],
                                  osems.at[c]) for c in range(NQ)]
    for c in range(QF):
        cp_o[c].start()

    @pl.when(pl.program_id(0) >= 0)
    def _():
        for c in range(QF, NQ):
            a = at_flat(c * TQ, TQ, KS, 2 * D - KS)
            ot = part_ref[:, pl.ds((c - QF) * TQ, TQ)] + jnp.dot(
                wot_ref[:, pl.ds(KS, 2 * D - KS)], a, preferred_element_type=F32)
            out_ref[:, pl.ds(c * TQ, TQ)] = ot.astype(out_ref.dtype)
            cp_o[c].start()
    for c in range(NQ):
        cp_o[c].wait()


@jax.jit
def pallas_gated_mix__mha_block__mha_block__prompt_kernel(
    A_x, A_wqkv, A_wo, B_x, B_wqkv, B_wo, gate_w,
):
    scratch = [
        pltpu.VMEM((D, S), BF16),
        pltpu.VMEM((2, D, 3 * D), BF16),
        pltpu.VMEM((2 * D, D), BF16),
        pltpu.VMEM((D,), BF16),
        pltpu.VMEM((D, S), BF16),
        pltpu.SemaphoreType.DMA((5 + NQ,)),
        pltpu.SemaphoreType.DMA((NQ,)),
        pltpu.VMEM((2, 3 * D, D), BF16),
        pltpu.VMEM((D, 2 * D), BF16),
        pltpu.VMEM((2 * H, HP, S), BF16),
        pltpu.VMEM((2 * H, S, HP), BF16),
        pltpu.VMEM((2 * H, HP, S), BF16),
        pltpu.VMEM((H, 2 * DH, S), F32),
        pltpu.VMEM((D, G // 2 * TQ), F32),
        pltpu.VMEM((2, 8, S), F32),
        pltpu.VMEM((2, G, 8, TQ), F32),
    ] + [pltpu.VMEM((G, S, TQ), F32)] * 2
    hbm = lambda a: pltpu.with_memory_space_constraint(a, pltpu.HBM)
    out_t = pl.pallas_call(
        _kernel,
        out_shape=pltpu.HBM((1, D, S), BF16),
        grid=(1,),
        in_specs=[pl.BlockSpec(memory_space=pltpu.HBM)] * 6,
        out_specs=pl.BlockSpec(memory_space=pltpu.HBM),
        scratch_shapes=scratch,
        compiler_params=pltpu.CompilerParams(vmem_limit_bytes=120 * 1024 * 1024),
        name="gated_mix_mha",
    )(hbm(A_x.transpose(0, 2, 1)), hbm(A_wqkv), hbm(A_wo), hbm(B_wqkv), hbm(B_wo), hbm(gate_w))
    return out_t.transpose(0, 2, 1)
```

```python
import numpy as np
import jax
import jax.numpy as jnp
import jax.experimental.pallas as pl
import jax.experimental.pallas.tpu as pltpu

S, D, H, DH = 2048, 448, 16, 28
HP = 32
TQ = 512
KC = 128
G = 4
NQ = S // TQ
NJ = S // KC
NI = 2 * H * NQ
NB = NI // G
QF = NQ - G // 2
KS = (2 * H - 2) * DH // 128 * 128
QSCALE = float(DH ** -0.5 * np.log2(np.e))
F32 = jnp.float32
BF16 = jnp.bfloat16


def _kernel(x_hbm, wa_hbm, woa_hbm, wb_hbm, wob_hbm, gw_hbm, out_hbm,
            x_ref, w_ref, wo_ref, gw_ref, out_ref, sems, osems,
            wt_ref, wot_ref, qt_ref, k_ref, vt_ref, at_ref, part_ref,
            g_ref, m_ref, s0_ref, s1_ref):
    cp_w = [pltpu.make_async_copy(w, w_ref.at[i], sems.at[i]) for i, w in enumerate((wa_hbm, wb_hbm))]
    cp_x = [pltpu.make_async_copy(x_hbm.at[0, :, pl.ds(c * TQ, TQ)], x_ref.at[:, pl.ds(c * TQ, TQ)],
                                  sems.at[2 + c]) for c in range(NQ)]
    cp_g = pltpu.make_async_copy(gw_hbm, gw_ref, sems.at[2 + NQ])
    cp_wo = [pltpu.make_async_copy(w, wo_ref.at[pl.ds(i * D, D), :], sems.at[3 + NQ + i])
             for i, w in enumerate((woa_hbm, wob_hbm))]
    cp_w[0].start()
    cp_g.start()
    cp_x[0].start()

    def prep_w(blk):
        for j in range(pl.cdiv(3 * D, 128)):
            c0 = j * 128
            cw = min(128, 3 * D - c0)
            wt_ref[blk, pl.ds(c0, cw), :] = w_ref[blk, :, pl.ds(c0, cw)].astype(F32).T.astype(BF16)

    zpad = jnp.zeros((HP - DH, TQ), F32)
    opad = jnp.where(jax.lax.broadcasted_iota(jnp.int32, (HP - DH, TQ), 0) == 0, 1.0, 0.0).astype(F32)

    def project(blk, c):
        q0 = c * TQ if isinstance(c, int) else pl.multiple_of(c * TQ, TQ)
        xs = x_ref[:, pl.ds(q0, TQ)]
        k = jnp.dot(wt_ref[blk, pl.ds(D, D), :], xs, preferred_element_type=F32)
        for hg in range(H // 4):
            kg = jnp.concatenate(
                [z for h in range(4 * hg, 4 * hg + 4) for z in (k[h * DH:(h + 1) * DH], zpad)], axis=0)
            kg = kg.T.astype(BF16)
            for hh in range(4):
                k_ref[blk * H + 4 * hg + hh, pl.ds(q0, TQ), :] = kg[:, hh * HP:(hh + 1) * HP]
        q = jnp.dot(wt_ref[blk, pl.ds(0, D), :], xs, preferred_element_type=F32) * QSCALE
        v = jnp.dot(wt_ref[blk, pl.ds(2 * D, D), :], xs, preferred_element_type=F32)
        for h in range(H):
            qh = jnp.concatenate([q[h * DH:(h + 1) * DH], zpad], axis=0)
            qt_ref[blk * H + h, :, pl.ds(q0, TQ)] = qh.astype(BF16)
            vh = jnp.concatenate([v[h * DH:(h + 1) * DH], opad], axis=0)
            vt_ref[blk * H + h, :, pl.ds(q0, TQ)] = vh.astype(BF16)

    cp_w[0].wait()
    cp_w[1].start()
    for c in cp_x[1:]:
        c.start()
    prep_w(0)
    cp_g.wait()
    cp_x[0].wait()
    project(0, 0)
    cp_w[1].wait()
    for c in cp_x[1:]:
        c.wait()
    for c in cp_wo:
        c.start()
    project(0, 1)
    gw16 = jnp.broadcast_to(gw_ref[...].reshape(1, D), (16, D))
    gpre = jnp.dot(gw16, x_ref[...], preferred_element_type=F32)[0:8, :]
    gate = 1.0 / (1.0 + jnp.exp(-gpre))
    g_ref[0] = gate
    g_ref[1] = 1.0 - gate
    prep_w(1)

    def pbody(t, carry):
        project(t // NQ, t % NQ)
        return carry
    jax.lax.fori_loop(2, 2 * NQ, pbody, 0)

    def idx(i):
        h = 2 * (i // (2 * NQ)) + i % 2
        return h, pl.multiple_of((i // 2) % NQ * TQ, TQ)

    def qk_chunk(h, qt, j, buf):
        s = jnp.dot(k_ref[h, pl.ds(j * KC, KC), :], qt, preferred_element_type=F32)
        buf[pl.ds(j * KC, KC), :] = s
        return s.reshape(KC // 8, 8, TQ).max(axis=0)

    def pv_chunk(h, m, j, buf):
        p = jnp.exp2(buf[pl.ds(j * KC, KC), :] - m).astype(BF16)
        return jnp.dot(vt_ref[h, :, pl.ds(j * KC, KC)], p, preferred_element_type=F32)

    bufs = (s0_ref, s1_ref)
    for c in cp_wo:
        c.wait()
    for g in range(G):
        h0, q00 = idx(g)
        qt = qt_ref[h0, :, pl.ds(q00, TQ)]
        m = None
        for j in range(NJ):
            mm = qk_chunk(h0, qt, j, bufs[0].at[g])
            m = mm if m is None else jnp.maximum(m, mm)
        m_ref[0, g] = m
    for j in range(2 * D // 128):
        wot_ref[:, pl.ds(j * 128, 128)] = wo_ref[pl.ds(j * 128, 128), :].astype(F32).T.astype(BF16)

    def at_flat(c0, w, r0, n):
        lo, hi = r0 // (2 * DH), pl.cdiv(r0 + n, 2 * DH)
        a = at_ref[pl.ds(lo, hi - lo), :, pl.ds(c0, w)].reshape((hi - lo) * 2 * DH, w)
        return a[r0 - lo * 2 * DH:r0 - lo * 2 * DH + n].astype(BF16)

    def block(b, par, do_qk=True):
        for g in range(G):
            i = b * G + g
            h, q0 = idx(i)
            cur = bufs[par].at[g]
            nxt = bufs[1 - par].at[g]
            if do_qk:
                hn, qn = idx(i + G)
                qt = qt_ref[hn, :, pl.ds(qn, TQ)]
            m = jnp.max(m_ref[par, g], axis=0, keepdims=True)
            mn = None
            acc = None
            qk_first = g < G - 1
            for j in range(NJ):
                if do_qk and qk_first:
                    mm = qk_chunk(hn, qt, j, nxt)
                    mn = mm if mn is None else jnp.maximum(mn, mm)
                pv = pv_chunk(h, m, j, cur)
                acc = pv if acc is None else acc + pv
                if do_qk and not qk_first:
                    mm = qk_chunk(hn, qt, j, nxt)
                    mn = mm if mn is None else jnp.maximum(mn, mm)
                npc = S // 128 // G
                if not do_qk and j % (NJ // npc) == 0:
                    c0 = (g * npc + j // (NJ // npc)) * 128
                    if c0 < QF * TQ:
                        out_ref[:, pl.ds(c0, 128)] = jnp.dot(
                            wot_ref[...], at_flat(c0, 128, 0, 2 * D),
                            preferred_element_type=F32).astype(out_ref.dtype)
                    else:
                        part_ref[:, pl.ds(c0 - QF * TQ, 128)] = jnp.dot(
                            wot_ref[:, pl.ds(0, KS)], at_flat(c0, 128, 0, KS),
                            preferred_element_type=F32)
            gt = g_ref[h // H, 0:1, pl.ds(q0, TQ)]
            at_ref[h // 2, pl.ds(g % 2 * DH, DH), pl.ds(q0, TQ)] = acc[0:DH] * (gt / acc[DH:DH + 1, :])
            if do_qk:
                m_ref[1 - par, g] = mn

    def body(b, c):
        @pl.when(b % 2 == 0)
        def _():
            block(b, 0)

        @pl.when(b % 2 == 1)
        def _():
            block(b, 1)
        return c
    jax.lax.fori_loop(0, NB - 1, body, 0)
    block(NB - 1, (NB - 1) % 2, do_qk=False)

    cp_o = [pltpu.make_async_copy(out_ref.at[:, pl.ds(c * TQ, TQ)], out_hbm.at[0, :, pl.ds(c * TQ, TQ)],
                                  osems.at[c]) for c in range(NQ)]
    for c in range(QF):
        cp_o[c].start()

    @pl.when(pl.program_id(0) >= 0)
    def _():
        for c in range(QF, NQ):
            ot = part_ref[:, pl.ds((c - QF) * TQ, TQ)] + jnp.dot(
                wot_ref[:, pl.ds(KS, 2 * D - KS)], at_flat(c * TQ, TQ, KS, 2 * D - KS),
                preferred_element_type=F32)
            out_ref[:, pl.ds(c * TQ, TQ)] = ot.astype(out_ref.dtype)
            cp_o[c].start()
    for c in range(NQ):
        cp_o[c].wait()


@jax.jit
def pallas_gated_mix__mha_block__mha_block__prompt_kernel(
    A_x, A_wqkv, A_wo, B_x, B_wqkv, B_wo, gate_w,
):
    del B_x
    scratch = [
        pltpu.VMEM((D, S), BF16),
        pltpu.VMEM((2, D, 3 * D), BF16),
        pltpu.VMEM((2 * D, D), BF16),
        pltpu.VMEM((D,), BF16),
        pltpu.VMEM((D, S), BF16),
        pltpu.SemaphoreType.DMA((5 + NQ,)),
        pltpu.SemaphoreType.DMA((NQ,)),
        pltpu.VMEM((2, 3 * D, D), BF16),
        pltpu.VMEM((D, 2 * D), BF16),
        pltpu.VMEM((2 * H, HP, S), BF16),
        pltpu.VMEM((2 * H, S, HP), BF16),
        pltpu.VMEM((2 * H, HP, S), BF16),
        pltpu.VMEM((H, 2 * DH, S), F32),
        pltpu.VMEM((D, G // 2 * TQ), F32),
        pltpu.VMEM((2, 8, S), F32),
        pltpu.VMEM((2, G, 8, TQ), F32),
        pltpu.VMEM((G, S, TQ), F32),
        pltpu.VMEM((G, S, TQ), F32),
    ]
    out_t = pl.pallas_call(
        _kernel,
        out_shape=jax.ShapeDtypeStruct((1, D, S), BF16),
        grid=(1,),
        in_specs=[pl.BlockSpec(memory_space=pltpu.HBM)] * 6,
        out_specs=pl.BlockSpec(memory_space=pltpu.HBM),
        scratch_shapes=scratch,
        compiler_params=pltpu.CompilerParams(vmem_limit_bytes=120 * 1024 * 1024),
        name="gated_mix_mha",
    )(A_x.transpose(0, 2, 1), A_wqkv, A_wo, B_wqkv, B_wo, gate_w)
    return out_t.transpose(0, 2, 1)
```
